```python
import os as _os
_os.environ.setdefault("JAX_PLATFORMS", "cpu")
import jax
import jax.numpy as jnp

def _softmax(x, axis=-1):
    return jax.nn.softmax(x, axis=axis)
def _gelu(x):
    return jax.nn.gelu(x, approximate=True)
def _silu(x):
    return jax.nn.silu(x)
def _sigmoid(x):
    return jax.nn.sigmoid(x)
def _layernorm(x, axis=-1, eps=1e-5):
    m = jnp.mean(x, axis=axis, keepdims=True)
    v = jnp.var(x, axis=axis, keepdims=True)
    return (x - m) / jnp.sqrt(v + eps)
def _scatter_add(tgt, idx, src, axis=0):
    return tgt.at[idx].add(src)
def _segment_sum(src, seg, n):
    return jax.ops.segment_sum(src, seg, n)
class _Rng:
    def __init__(self, key):
        self._k = key
    def _next(self):
        self._k, sub = jax.random.split(self._k)
        return sub
    def normal(self, shape):
        return jax.random.normal(self._next(), shape, dtype=jnp.bfloat16)
    def randint(self, lo, hi, shape):
        return jax.random.randint(self._next(), shape, lo, hi, dtype=jnp.int32)
    def uniform(self, shape, lo=0.0, hi=1.0):
        return jax.random.uniform(self._next(), shape, jnp.bfloat16, lo, hi)
    def permutation(self, n):
        return jax.random.permutation(self._next(), n)


kernel_name = 'gated_mix__mha_block_cached__swiglu_ffn__decode'

def setup_inputs():
    _rng = _Rng(jax.random.key(int.from_bytes(__import__("os").urandom(4), "little")))
    _w = (lambda a: (lambda t: t.astype(jnp.bfloat16) if jnp.issubdtype(t.dtype, jnp.floating) else t)(jnp.asarray(a)))
    def _A_setup():
        B, Sq, D = 4, 1, 512
        H, Sk, Dh = 32, 4096, 128
        return {
            "x": _w((lambda *s: _rng.normal(s) * 0.05)(B, Sq, D)),
            "k_cache": _w((lambda *s: _rng.normal(s) * 3.2)(B, H, Sk, Dh)),
            "v_cache": _w((lambda *s: _rng.normal(s) * 0.4)(B, H, Sk, Dh)),
            "wq": _w((lambda *s: _rng.normal(s) * 3.2)(D, H * Dh) * (D ** -0.5)),
            "wo": _w((lambda *s: _rng.normal(s) * 0.4)(H * Dh, D) * ((H * Dh) ** -0.5)),
        }
    _A_in = _A_setup()

    def _B_setup():
        B, S, D, F = 4, 1, 512, 1376
        return {
            "x": _w((lambda *s: _rng.normal(s) * 0.05)(B, S, D)),
            "w_gate": _w((lambda *s: _rng.normal(s) * 0.05)(D, F)),
            "w_up": _w((lambda *s: _rng.normal(s) * 0.05)(D, F)),
            "w_down": _w((lambda *s: _rng.normal(s) * 0.05)(F, D)),
        }
    _B_in = _B_setup()

    return {
        "A_x": _A_in["x"],
        "A_k_cache": _A_in["k_cache"],
        "A_v_cache": _A_in["v_cache"],
        "A_wq": _A_in["wq"],
        "A_wo": _A_in["wo"],
        "B_x": _B_in["x"],
        "B_w_gate": _B_in["w_gate"],
        "B_w_up": _B_in["w_up"],
        "B_w_down": _B_in["w_down"],
        "gate_w": _w((lambda *s: _rng.normal(s) * 0.05)(512) * 16.0),
    }

def reference(A_x, A_k_cache, A_v_cache, A_wq, A_wo, B_x, B_w_gate, B_w_up, B_w_down, gate_w):
    def _A_ref(x, k_cache, v_cache, wq, wo):
        B, Sq, D = x.shape
        H, Dh = 32, 128
        q = (lambda x, *d: x.transpose(*d))((x @ wq).reshape(B, Sq, H, Dh), 0, 2, 1, 3)
        scores = jnp.einsum("bhqd,bhkd->bhqk", q, k_cache) * (Dh ** -0.5)
        p = _softmax(scores, axis=-1)
        o = jnp.einsum("bhqk,bhkd->bhqd", p, v_cache)
        return (lambda x, *d: x.transpose(*d))(o, 0, 2, 1, 3).reshape(B, Sq, H * Dh) @ wo

    def _B_ref(x, w_gate, w_up, w_down):
        g = _silu(x @ w_gate)
        u = x @ w_up
        return (g * u) @ w_down

    x = A_x
    g = _sigmoid((x * gate_w).sum(-1, keepdims=True))
    a = _A_ref(x, A_k_cache, A_v_cache, A_wq, A_wo)
    b = _B_ref(x, B_w_gate, B_w_up, B_w_down)
    return g * a + (1 - g) * b
```

```python
import functools
import jax
import jax.numpy as jnp
from jax import lax
import jax.experimental.pallas as pl
import jax.experimental.pallas.tpu as pltpu

B, D, H, SK, DH, F = 4, 512, 32, 4096, 128, 1376
NT = (((1,), (1,)), ((), ()))


def _make(nslot=3, wo_chunks=(2048, 1024, 512, 256, 128, 128), params=None, name="gated_mix_decode"):
    params = params or {}
    assert sum(wo_chunks) == H * DH

    def body(x_hbm, k_hbm, v_hbm, wq_hbm, wo_hbm, wg_hbm, wu_hbm, wd_hbm, gw_hbm, out_hbm,
             x_v, gw_v, wq_v, wo_v, wg_v, wu_v, wd_v, kbuf, vbuf, q_s, o_s, out_v,
             ksem, vsem, wsem, osem):
        def k_copy(i, slot):
            return pltpu.make_async_copy(k_hbm.at[i], kbuf.at[slot], ksem.at[slot])

        def v_copy(i, slot):
            return pltpu.make_async_copy(v_hbm.at[i], vbuf.at[slot], vsem.at[slot])

        half = D // 2
        cp_wq0 = pltpu.make_async_copy(wq_hbm.at[pl.ds(0, half)], wq_v.at[pl.ds(0, half)], wsem.at[0])
        cp_wq1 = pltpu.make_async_copy(wq_hbm.at[pl.ds(half, half)], wq_v.at[pl.ds(half, half)], wsem.at[1])
        cp_x = pltpu.make_async_copy(x_hbm, x_v, wsem.at[2])
        cp_gw = pltpu.make_async_copy(gw_hbm, gw_v, wsem.at[3])
        cp_wg = pltpu.make_async_copy(wg_hbm, wg_v, wsem.at[4])
        cp_wu = pltpu.make_async_copy(wu_hbm, wu_v, wsem.at[5])
        cp_wd = pltpu.make_async_copy(wd_hbm, wd_v, wsem.at[6])
        cp_wo = []
        r = 0
        for j, n in enumerate(wo_chunks):
            cp_wo.append((r, n, pltpu.make_async_copy(wo_hbm.at[pl.ds(r, n)], wo_v.at[pl.ds(r, n)], osem.at[j])))
            r += n

        cp_wq0.start(priority=0)
        cp_wq1.start(priority=1)
        cp_x.start(priority=0)
        cp_gw.start(priority=1)
        cp_wg.start(priority=0)
        cp_wu.start(priority=1)
        cp_wd.start(priority=0)
        for s in range(nslot):
            k_copy(s, s).start(priority=0)
            v_copy(s, s).start(priority=1)

        o_s[...] = jnp.zeros(o_s.shape, o_s.dtype)

        cp_x.wait()
        x = x_v[...]
        x8 = jnp.concatenate([x.astype(jnp.float32)] * 2, axis=0).astype(jnp.bfloat16)
        cp_wq0.wait()
        cp_wq1.wait()
        q = jnp.dot(x8, wq_v[...], preferred_element_type=jnp.float32)
        for h in range(H):
            q_s[h] = q[:, h * DH:(h + 1) * DH]

        cp_gw.wait()
        gw = gw_v[...].astype(jnp.float32)
        xf = x8.astype(jnp.float32)
        z = xf[:, 0:128] * gw[0:1, :]
        for c in range(1, 4):
            z = z + xf[:, c * 128:(c + 1) * 128] * gw[c:c + 1, :]
        gate = jax.nn.sigmoid(jnp.sum(z, axis=-1, keepdims=True))

        cp_wg.wait()
        cp_wu.wait()
        hg = lax.dot_general(x8, wg_v[...], NT, preferred_element_type=jnp.float32)
        hu = lax.dot_general(x8, wu_v[...], NT, preferred_element_type=jnp.float32)
        hh = (hg * jax.nn.sigmoid(hg) * hu).astype(jnp.bfloat16)
        cp_wd.wait()
        ffn = jnp.dot(hh, wd_v[...], preferred_element_type=jnp.float32)
        ffn = (1.0 - gate) * ffn

        scale = DH ** -0.5
        row = lax.broadcasted_iota(jnp.int32, (8, DH), 0)

        def head(i, prefetch):
            slot = i % nslot
            b = i // H
            h = i % H
            qh = q_s[h].astype(jnp.bfloat16)
            k_copy(i, slot).wait()
            s = lax.dot_general(qh, kbuf[slot], NT, preferred_element_type=jnp.float32) * scale
            if prefetch:
                k_copy(i + nslot, slot).start(priority=0)
            m = jnp.max(s, axis=-1, keepdims=True)
            p = jnp.exp(s - m)
            l = jnp.sum(p, axis=-1, keepdims=True)
            v_copy(i, slot).wait()
            o = jnp.dot(p.astype(jnp.bfloat16), vbuf[slot], preferred_element_type=jnp.float32)
            if prefetch:
                v_copy(i + nslot, slot).start(priority=1)
            o_s[h] = jnp.where(row == b, o / l, o_s[h])

        n = B * H

        def main(i, c):
            head(i, True)
            return c
        lax.fori_loop(0, n - nslot, main, 0)
        for j, (_, _, cp) in enumerate(cp_wo):
            cp.start(priority=j % 2)

        def tail(i, c):
            head(i, False)
            return c
        lax.fori_loop(n - nslot, n, tail, 0)

        acc = jnp.zeros((8, D), jnp.float32)
        for r, nr, cp in cp_wo:
            lhs = jnp.concatenate([o_s[h] for h in range(r // DH, (r + nr) // DH)], axis=-1).astype(jnp.bfloat16)
            cp.wait()
            acc = acc + jnp.dot(lhs, wo_v[pl.ds(r, nr), :], preferred_element_type=jnp.float32)
        res = gate * acc + ffn
        out_v[...] = res[0:B].astype(out_v.dtype)
        cp_out = pltpu.make_async_copy(out_v, out_hbm, wsem.at[7])
        cp_out.start()
        cp_out.wait()

    @jax.jit
    def pallas_gated_mix__mha_block_cached__swiglu_ffn__decode_kernel(A_x, A_k_cache, A_v_cache, A_wq, A_wo, B_x, B_w_gate, B_w_up, B_w_down, gate_w):
        hbm = pl.BlockSpec(memory_space=pltpu.HBM)
        bf = jnp.bfloat16
        out = pl.pallas_call(
            body,
            in_specs=[hbm] * 9,
            out_specs=hbm,
            out_shape=jax.ShapeDtypeStruct((B, D), bf),
            scratch_shapes=[
                pltpu.VMEM((B, D), bf), pltpu.VMEM((4, 128), bf),
                pltpu.VMEM((D, H * DH), bf), pltpu.VMEM((H * DH, D), bf),
                pltpu.VMEM((F, D), bf), pltpu.VMEM((F, D), bf), pltpu.VMEM((F, D), bf),
                pltpu.VMEM((nslot, SK, DH), bf), pltpu.VMEM((nslot, SK, DH), bf),
                pltpu.VMEM((H, 8, DH), jnp.float32), pltpu.VMEM((H, 8, DH), jnp.float32),
                pltpu.VMEM((B, D), bf),
                pltpu.SemaphoreType.DMA((nslot,)), pltpu.SemaphoreType.DMA((nslot,)),
                pltpu.SemaphoreType.DMA((8,)), pltpu.SemaphoreType.DMA((len(wo_chunks),)),
            ],
            compiler_params=pltpu.CompilerParams(vmem_limit_bytes=100 * 1024 * 1024, **params),
            name=name,
        )(A_x.reshape(B, D), A_k_cache.reshape(B * H, SK, DH), A_v_cache.reshape(B * H, SK, DH),
          A_wq, A_wo, B_w_gate.T, B_w_up.T, B_w_down, gate_w.reshape(4, 128))
        return out.reshape(B, 1, D)
    return pallas_gated_mix__mha_block_cached__swiglu_ffn__decode_kernel


pallas_gated_mix__mha_block_cached__swiglu_ffn__decode_kernel = _make()
```

```python
import functools
import jax
import jax.numpy as jnp
from jax import lax
import jax.experimental.pallas as pl
import jax.experimental.pallas.tpu as pltpu

B, D, H, SK, DH, F = 4, 512, 32, 4096, 128, 1376
NT = (((1,), (1,)), ((), ()))
NH = 4
NJ = H // NH
NS = B * NH
PR = 256
NP = SK // PR
SROWS = NJ * SK
NOCHK = dict(disable_bounds_checks=True, disable_semaphore_checks=True)


def _al(v, m):
    return v if isinstance(v, int) else pl.multiple_of(v, m)


def _make(r0=64, dk=64, dv=64, look=48, order=None, params=NOCHK, name="gated_mix_decode",
         compute=True, early=1, group=4, wlook=None, tail=((0, 64), (64, 64)), burst=True,
         last_group=None, mixw=True, qat=12):
    order = list(order or range(NS))
    L = 2 * NS
    last_group = last_group or group
    NSEM = 4 * L
    assert look <= 2 * L

    def body(x_hbm, k_hbm, v_hbm, wq_hbm, wo_hbm, wg_hbm, wu_hbm, wd_hbm, gw_hbm, out_hbm,
             x_v, gw_v, wq_v, wo_v, wg_v, wu_v, wd_v, kbuf, vbuf, q_s, s_s, f_s, out_v,
             sem, wsem, msem):

        def kv_entry(which, j, i, e):
            src, buf, d = ((k_hbm, kbuf, dk), (v_hbm, vbuf, dv))[which]
            n, c = order[e // 2], e % 2
            off, rows = ((0, r0), (r0, PR - r0))[c]
            r = i * PR + d + off
            return pltpu.make_async_copy(
                src.at[n % B, n // B, pl.ds(_al(j * SK + r, 16), rows)],
                buf.at[n, pl.ds(_al(r, 16), rows)],
                sem.at[(i % 4) * L + e]), c

        def kv_entry_end(which, e):
            src, buf, d = ((k_hbm, kbuf, dk), (v_hbm, vbuf, dv))[which]
            n, c = order[e // 2], e % 2
            off, rows = ((0, r0), (r0, PR - r0))[c]
            r = (NP - 1) * PR + d + off
            rows = min(rows, SK - r)
            if rows <= 0:
                return None, c
            return pltpu.make_async_copy(
                src.at[n % B, n // B, pl.ds((NJ - 1) * SK + r, rows)],
                buf.at[n, pl.ds(r, rows)],
                sem.at[((NP - 1) % 4) * L + e]), c

        def kv_do(op, which, j, i, e):
            def act(entry):
                cp, pr = entry
                if cp is not None:
                    cp.wait() if op == "wait" else cp.start(priority=pr)
            d = (dk, dv)[which]
            clipped = isinstance(i, int) and i == NP - 1 and d + ((r0, PR)[e % 2]) > PR
            if not clipped:
                act(kv_entry(which, j, i, e))
            else:
                pl.when(j < NJ - 1)(lambda: act(kv_entry(which, lax.min(j, NJ - 2), i, e)))
                pl.when(j == NJ - 1)(lambda: act(kv_entry_end(which, e)))

        def w_list(kind, u):
            out = []

            def add(src, dst, idx, pr):
                out.append((src.at[idx], dst.at[idx], pr))

            def ffn(t):
                rows = pl.ds(_al(t * 16, 16), 16)
                add(wu_hbm, wu_v, (pl.ds(0, 1), rows), 0)
                add(wg_hbm, wg_v, (pl.ds(0, 2), rows), 1)
                add(wu_hbm, wu_v, (pl.ds(1, 1), rows), 0)
                add(wd_hbm, wd_v, (pl.ds(0, 2), rows), 1)
            if kind < 2:
                t = u + (0, 24)[kind]
                rq = pl.ds(_al((t // 4) * 8, 8), 8)
                cq = pl.ds(_al((t % 4) * 1024, 1024), 1024)
                ro = pl.ds(_al(t * 16, 16), 16)
                for s in (0, 4):
                    add(wq_hbm, wq_v, (pl.ds(s, 1), rq, cq), 0)
                    add(wq_hbm, wq_v, (pl.ds(s + 1, 3), rq, cq), 1)
                for a in range(2 - kind):
                    add(wo_hbm, wo_v, (pl.ds(0, 1), a, ro), 0)
                    add(wo_hbm, wo_v, (pl.ds(1, 3), a, ro), 1)
                if mixw:
                    if kind == 0:
                        ffn(u)
                    else:
                        ffn(24 + 2 * u)
                        ffn(25 + 2 * u)
            elif kind == 3:
                ffn(u)
            else:
                if mixw:
                    for t in range(40, 43):
                        ffn(t)
                for src, buf, d in ((k_hbm, kbuf, dk), (v_hbm, vbuf, dv)):
                    if d:
                        for hh in range(NH):
                            out.append((src.at[pl.ds(0, 1), hh, pl.ds(0, d)], buf.at[pl.ds(hh * B, 1), pl.ds(0, d)], 0))
                            out.append((src.at[pl.ds(1, 3), hh, pl.ds(0, d)], buf.at[pl.ds(hh * B + 1, 3), pl.ds(0, d)], 1))
            return out

        sections = [(0, 24), (1, 8)] + ([] if mixw else [(3, 43)]) + [(2, 1)]
        lens = [len(w_list(k, 0)) for k, _ in sections]
        starts = [sum(l * n for l, (_, n) in zip(lens[:s], sections[:s])) for s in range(len(sections) + 1)]
        NW = starts[-1]
        wl = wlook or look
        WS = 64
        assert wl <= WS

        def w_entry(s, u, e):
            src, dst, pr = w_list(sections[s][0], u)[e]
            return pltpu.make_async_copy(src, dst, wsem.at[(starts[s] + u * lens[s] + e) % WS]), pr

        def start_global(t):
            if t < NW:
                s = max(k for k in range(len(sections)) if starts[k] <= t)
                cp, pr = w_entry(s, (t - starts[s]) // lens[s], (t - starts[s]) % lens[s])
                cp.start(priority=pr)
            else:
                kv_do("start", 0, 0, (t - NW) // L, (t - NW) % L)

        def tail_copy(t):
            a, n = tail[t // 2]
            hs = (pl.ds(0, 1), pl.ds(1, 3))[t % 2]
            idx = (hs, 1, pl.ds(384 + a, n))
            return pltpu.make_async_copy(wo_hbm.at[idx], wo_v.at[idx], wsem.at[t])

        cp_x = pltpu.make_async_copy(x_hbm, x_v, msem.at[0])
        cp_gw = pltpu.make_async_copy(gw_hbm, gw_v, msem.at[1])
        for t in range(wl):
            start_global(t)
        cp_x.start()
        cp_gw.start()
        issued = wl
        for s, (kind, n) in enumerate(sections):
            l = lens[s]
            nloop = max(0, n - -(-wl // l))

            def w_iter(u, c, s=s, l=l):
                for e in range(l):
                    w_entry(s, u, e)[0].wait()
                    cp, pr = w_entry(s, u + (e + wl) // l, (e + wl) % l)
                    cp.start(priority=pr)
                return c
            if nloop:
                lax.fori_loop(0, nloop, w_iter, 0)
                issued += nloop * l
            for u in range(nloop, n):
                for e in range(l):
                    w_entry(s, u, e)[0].wait()
                    t = starts[s] + u * l + e
                    target = t + wl + 1 if t + 1 < NW else NW + look
                    while issued < min(target, NW + look):
                        start_global(issued)
                        issued += 1
        assert issued == NW + look

        cp_x.wait()
        cp_gw.wait()
        xf = x_v[...].astype(jnp.float32)
        xf = jnp.concatenate([xf, xf], axis=0)
        x8 = xf.astype(jnp.bfloat16)
        row = lax.broadcasted_iota(jnp.int32, (8, DH), 0)
        def q_job(j):
            for g in range(2):
                qq = []
                for e in range(2):
                    cols = pl.ds(_al(((2 * g + e) * NJ + j) * DH, DH), DH)
                    qq.append(jnp.dot(x8, wq_v[:, :, cols].reshape(D, DH), preferred_element_type=jnp.float32))
                q_s[j, g] = jnp.where(row < B, qq[0], qq[1])

        def ffn_job(i):
            half, c = i // 6, i % 6
            lo = lax.min(c * DH, F // 2 - DH)
            rows = pl.ds(pl.multiple_of(lo, 16), DH)
            hg = lax.dot_general(x8, wg_v[half, rows, :], NT, preferred_element_type=jnp.float32)
            hu = lax.dot_general(x8, wu_v[half, rows, :], NT, preferred_element_type=jnp.float32)
            hid = hg * jax.nn.sigmoid(hg) * hu
            col = lax.broadcasted_iota(jnp.int32, (8, DH), 1)
            hid = jnp.where(col >= c * DH - lo, hid, 0.0).astype(jnp.bfloat16)
            f_s[...] += jnp.dot(hid, wd_v[half, rows, :], preferred_element_type=jnp.float32)

        f_s[...] = jnp.zeros(f_s.shape, f_s.dtype)
        if burst:
            q_job(0)
        gw = gw_v[...].astype(jnp.float32)
        z = xf[:, 0:128] * gw[0:1, :]
        for c in range(1, 4):
            z = z + xf[:, c * 128:(c + 1) * 128] * gw[c:c + 1, :]
        gate = jax.nn.sigmoid(jnp.sum(z, axis=-1, keepdims=True))

        scale = DH ** -0.5
        rowp = lax.broadcasted_iota(jnp.int32, (8, PR), 0)

        def period(which, j, i, work, grp):
            buf = (kbuf, vbuf)[which]
            pos = 0
            for s0 in range(0, NS, grp):
                while pos < min(L, 2 * (s0 + grp) + early):
                    kv_do("wait", which, j, i, pos)
                    di, e = divmod(pos + look, L)
                    if not isinstance(i, int) or i + di < NP:
                        kv_do("start", which, j, i + di, e)
                    elif which == 0:
                        kv_do("start", 1, j, i + di - NP, e)
                    else:
                        t = (i + di - NP) * L + e
                        pl.when(j < NJ - 1)(functools.partial(kv_do, "start", 0, lax.min(j + 1, NJ - 1), i + di - NP, e))
                        if t < 2 * len(tail):
                            pl.when(j == NJ - 1)(functools.partial(tail_copy(t).start, priority=t % 2))
                    pos += 1
                if compute:
                    for n in order[s0:s0 + grp]:
                        work(n, buf[n, pl.ds(_al(i * PR, PR), PR), :])

        def k_period(j, i, qs, mrun):
            sc = [None, None]

            def work(n, val):
                g, r = divmod(n, 8)
                res = lax.dot_general(qs[g], val, NT, preferred_element_type=jnp.float32)
                sc[g] = res if sc[g] is None else jnp.where(rowp == r, res, sc[g])
            period(0, j, i, work, group)
            if burst and not isinstance(i, int):
                pl.when(jnp.logical_and(j == 0, i < 12))(lambda: ffn_job(i))
                pl.when(jnp.logical_and(j < NJ - 1, i == qat))(lambda: q_job(lax.min(j + 1, NJ - 1)))
            if not compute:
                return mrun
            new = []
            for g in range(2):
                s = sc[g] * scale
                s_s[i, g] = s
                m = mrun[g]
                for c in range(PR // DH):
                    m = jnp.maximum(m, s[:, c * DH:(c + 1) * DH])
                new.append(m)
            return tuple(new)

        def v_period(j, i, ms, carry, grp):
            lrun, acc = carry
            if not compute:
                period(1, j, i, None, grp)
                return carry
            ps, lnew = [], []
            for g in range(2):
                p = jnp.exp(s_s[i, g] - ms[g])
                l = lrun[g]
                for c in range(PR // DH):
                    l = l + p[:, c * DH:(c + 1) * DH]
                lnew.append(l)
                ps.append(p.astype(jnp.bfloat16))
            oc = [None, None]

            def work(n, val):
                g, r = divmod(n, 8)
                res = jnp.dot(ps[g], val, preferred_element_type=jnp.float32)
                oc[g] = res if oc[g] is None else jnp.where(row == r, res, oc[g])
            period(1, j, i, work, grp)
            return tuple(lnew), tuple(acc[g] + oc[g] for g in range(2))

        def carry_over(buf, d):
            if d and compute:
                buf[:, pl.ds(0, d), :] = buf[:, pl.ds(SK, d), :]

        def head_lhs(lrun, acc):
            parts = []
            for g in range(2):
                o = acc[g] / jnp.sum(lrun[g], axis=-1, keepdims=True)
                parts += [jnp.where(row < B, o, 0.0), jnp.where(row < B, 0.0, o)]
            return parts

        nloop = NP - 3

        def super_block(j, carry):
            y, _ = carry
            qs = [q_s[j, g].astype(jnp.bfloat16) for g in range(2)]
            ninf = jnp.full((8, DH), -jnp.inf, jnp.float32)
            zero = jnp.zeros((8, DH), jnp.float32)
            mrun = lax.fori_loop(0, nloop, lambda i, m: k_period(j, i, qs, m), (ninf, ninf))
            for i in range(nloop, NP):
                mrun = k_period(j, i, qs, mrun)
            carry_over(kbuf, dk)
            ms = [jnp.max(m, axis=-1, keepdims=True) for m in mrun]
            c = ((zero, zero), (zero, zero))
            c = lax.fori_loop(0, nloop, lambda i, c: v_period(j, i, ms, c, group), c)
            for i in range(nloop, NP):
                c = v_period(j, i, ms, c, last_group if i == NP - 1 else group)
            carry_over(vbuf, dv)
            parts = head_lhs(*c)

            def project(y):
                jj = lax.min(j, NJ - 2)
                rows = pl.ds(pl.multiple_of((jj % 4) * DH, DH), DH)
                w = wo_v[:, jj // 4, rows, :].reshape(NH * DH, D)
                lhs = jnp.concatenate(parts, axis=-1).astype(jnp.bfloat16)
                return y + jnp.dot(lhs, w, preferred_element_type=jnp.float32)
            y = lax.cond(j < NJ - 1, project, lambda y: y, y)
            return y, tuple(parts)

        zero = jnp.zeros((8, DH), jnp.float32)
        y, parts = lax.fori_loop(0, NJ, super_block, (jnp.zeros((8, D), jnp.float32), (zero,) * NH))
        q_s[0, 0] = y[:, 0:128]
        for t, (a, n) in enumerate(tail):
            lhs = jnp.concatenate([p[:, a:a + n] for p in parts], axis=-1).astype(jnp.bfloat16)
            tail_copy(2 * t).wait()
            tail_copy(2 * t + 1).wait()
            w = wo_v[:, 1, pl.ds(384 + a, n), :].reshape(NH * n, D)
            y = y + jnp.dot(lhs, w, preferred_element_type=jnp.float32)
            if t + 1 < len(tail):
                s_s[0, 0] = y[:, 0:PR]
        res = gate[0:B] * (y[0:B] + y[B:2 * B]) + (1.0 - gate[0:B]) * f_s[0:B]
        out_v[...] = res.astype(out_v.dtype)
        cp_out = pltpu.make_async_copy(out_v, out_hbm, msem.at[2])
        cp_out.start()
        cp_out.wait()

    @jax.jit
    def pallas_gated_mix__mha_block_cached__swiglu_ffn__decode_kernel(A_x, A_k_cache, A_v_cache, A_wq, A_wo, B_x, B_w_gate, B_w_up, B_w_down, gate_w):
        hbm = pl.BlockSpec(memory_space=pltpu.HBM)
        bf = jnp.bfloat16
        ffn_shape = (2, F // 2, D)
        out = pl.pallas_call(
            body,
            in_specs=[hbm] * 9,
            out_specs=hbm,
            out_shape=jax.ShapeDtypeStruct((B, D), bf),
            scratch_shapes=[
                pltpu.VMEM((B, D), bf), pltpu.VMEM((4, 128), bf),
                pltpu.VMEM((8, D // 8, H * DH), bf), pltpu.VMEM((NH, 2, 512, D), bf),
                pltpu.VMEM(ffn_shape, bf), pltpu.VMEM(ffn_shape, bf), pltpu.VMEM(ffn_shape, bf),
                pltpu.VMEM((NS, SK + max(dk, 16), DH), bf), pltpu.VMEM((NS, SK + max(dv, 16), DH), bf),
                pltpu.VMEM((NJ, 2, 8, DH), jnp.float32),
                pltpu.VMEM((NP, 2, 8, PR), jnp.float32),
                pltpu.VMEM((8, D), jnp.float32),
                pltpu.VMEM((B, D), bf),
                pltpu.SemaphoreType.DMA((NSEM,)),
                pltpu.SemaphoreType.DMA((64,)),
                pltpu.SemaphoreType.DMA((3,)),
            ],
            compiler_params=pltpu.CompilerParams(vmem_limit_bytes=100 * 1024 * 1024, **params),
            name=name,
        )(A_x.reshape(B, D), A_k_cache.reshape(B, NH, SROWS, DH), A_v_cache.reshape(B, NH, SROWS, DH),
          A_wq.reshape(8, D // 8, H * DH), A_wo.reshape(NH, 2, 512, D),
          B_w_gate.T.reshape(ffn_shape), B_w_up.T.reshape(ffn_shape), B_w_down.reshape(ffn_shape),
          gate_w.reshape(4, 128))
        return out.reshape(B, 1, D)
    return pallas_gated_mix__mha_block_cached__swiglu_ffn__decode_kernel


pallas_gated_mix__mha_block_cached__swiglu_ffn__decode_kernel = _make(wlook=32)
```

```python
import functools

import jax
import jax.numpy as jnp
from jax import lax
import jax.experimental.pallas as pl
import jax.experimental.pallas.tpu as pltpu

B, D, H, SK, DH, F = 4, 512, 32, 4096, 128, 1376

NH = 4
NS = B * NH
NJ = H // NH
PR = 256
NP = SK // PR
SHORT = 64
SHIFT = 64
AHEAD = 24
JOB = 4
RING = 4
W_AHEAD = 16
W_RING = 64
WO_TAIL = (3, 1)

NT = (((1,), (1,)), ((), ()))
F32, BF16 = jnp.float32, jnp.bfloat16


def _aligned(i, n):
    return i if isinstance(i, int) else pl.multiple_of(i, n)


def _kernel(x_hbm, k_hbm, v_hbm, wq_hbm, wo_hbm, wg_hbm, wu_hbm, wd_hbm, gw_hbm, out_hbm,
            x_v, gw_v, wq_v, wo_v, wg_v, wu_v, wd_v, k_v, v_v, q_v, s_v, ffn_v, out_v,
            kv_sem, w_sem, io_sem):
    caches = ((k_hbm, k_v), (v_hbm, v_v))

    def cache_copy(kv, j, i, e, clip=False):
        hbm, vmem = caches[kv]
        n = e // 2
        r = i * PR + SHIFT + (0, SHORT)[e % 2]
        rows = SK - r if clip else (SHORT, PR - SHORT)[e % 2]
        return pltpu.make_async_copy(
            hbm.at[n % B, n // B, pl.ds(_aligned(j * SK + r, 16), rows)],
            vmem.at[n, pl.ds(_aligned(r, 16), rows)],
            kv_sem.at[(i % RING) * 2 * NS + e])

    def cache_op(op, kv, j, i, e):
        def run(j, clip):
            copy = cache_copy(kv, j, i, e, clip)
            copy.wait() if op == "wait" else copy.start(priority=e % 2)

        if isinstance(i, int) and i == NP - 1 and e % 2:
            pl.when(j < NJ - 1)(lambda: run(lax.min(j, NJ - 2), False))
            pl.when(j == NJ - 1)(lambda: run(NJ - 1, True))
        else:
            run(j, False)

    def wo_tail_copy(t):
        idx = (pl.ds(sum(WO_TAIL[:t]), WO_TAIL[t]), 1, pl.ds(3 * DH, DH))
        return pltpu.make_async_copy(wo_hbm.at[idx], wo_v.at[idx], w_sem.at[t])

    def dma(op, kv, j, i, e):
        di, e = divmod(e, 2 * NS)
        if not isinstance(i, int) or i + di < NP:
            cache_op(op, kv, j, i + di, e)
        elif kv == 0:
            cache_op(op, 1, j, i + di - NP, e)
        else:
            pl.when(j < NJ - 1)(
                functools.partial(cache_op, op, 0, lax.min(j + 1, NJ - 1), i + di - NP, e))
            t = (i + di - NP) * NS + e // 2
            if op == "start" and e % 2 and t < len(WO_TAIL):
                pl.when(j == NJ - 1)(lambda: wo_tail_copy(t).start(priority=1))

    def weight_slices(section, u):
        out = []

        def ffn(t):
            rows = pl.ds(_aligned(t * 16, 16), 16)
            out.append((wu_hbm, wu_v, (pl.ds(0, 1), rows)))
            out.append((wg_hbm, wg_v, (pl.ds(0, 2), rows)))
            out.append((wu_hbm, wu_v, (pl.ds(1, 1), rows)))
            out.append((wd_hbm, wd_v, (pl.ds(0, 2), rows)))

        if section < 2:
            t = u + (0, 24)[section]
            q_rows = pl.ds(_aligned((t // 4) * 8, 8), 8)
            q_cols = pl.ds(_aligned((t % 4) * 1024, 1024), 1024)
            o_rows = pl.ds(_aligned(t * 16, 16), 16)
            for s in (0, 4):
                out.append((wq_hbm, wq_v, (pl.ds(s, 1), q_rows, q_cols)))
                out.append((wq_hbm, wq_v, (pl.ds(s + 1, 3), q_rows, q_cols)))
            for half in range(2 - section):
                out.append((wo_hbm, wo_v, (pl.ds(0, 1), half, o_rows)))
                out.append((wo_hbm, wo_v, (pl.ds(1, 3), half, o_rows)))
            for t in ((u,), (24 + 2 * u, 25 + 2 * u))[section]:
                ffn(t)
        else:
            for t in range(40, F // 32):
                ffn(t)
        out = [(src.at[idx], dst.at[idx]) for src, dst, idx in out]
        if section == 2:
            for hbm, vmem in caches:
                for hh in range(NH):
                    for b, nb in ((0, 1), (1, B - 1)):
                        out.append((hbm.at[pl.ds(b, nb), hh, pl.ds(0, SHIFT)],
                                    vmem.at[pl.ds(hh * B + b, nb), pl.ds(0, SHIFT)]))
        return out

    steps = (24, 8, 1)
    width = [len(weight_slices(s, 0)) for s in range(3)]
    first = [sum(w * n for w, n in zip(width[:s], steps[:s])) for s in range(4)]
    n_weight = first[-1]

    def weight_copy(section, u, e):
        src, dst = weight_slices(section, u)[e]
        return pltpu.make_async_copy(
            src, dst, w_sem.at[(first[section] + u * width[section] + e) % W_RING])

    def start_nth(t):
        if t < n_weight:
            s = max(k for k in range(3) if first[k] <= t)
            weight_copy(s, *divmod(t - first[s], width[s])).start(priority=t % 2)
        else:
            cache_op("start", 0, 0, *divmod(t - n_weight, 2 * NS))

    x_copy = pltpu.make_async_copy(x_hbm, x_v, io_sem.at[0])
    gw_copy = pltpu.make_async_copy(gw_hbm, gw_v, io_sem.at[1])
    for priority in (1, 0):
        for t in range(priority, 2 * W_AHEAD, 2):
            start_nth(t)
    x_copy.start()
    gw_copy.start()
    pending = [2 * W_AHEAD, 2 * W_AHEAD + 1]
    for s in range(3):
        looped = max(0, steps[s] - pl.cdiv(2 * W_AHEAD, width[s]))
        if looped:
            @pl.loop(0, looped)
            def _(u):
                for e in range(width[s]):
                    weight_copy(s, u, e).wait()
                    du, e2 = divmod(e + 2 * W_AHEAD, width[s])
                    weight_copy(s, u + du, e2).start(priority=e % 2)
            pending = [t + looped * width[s] for t in pending]
        for u in range(looped, steps[s]):
            for e in range(width[s]):
                weight_copy(s, u, e).wait()
                t = first[s] + u * width[s] + e
                upto = t + 2 * W_AHEAD if t + 2 < n_weight else n_weight + 2 * AHEAD - 1
                while pending[e % 2] <= upto:
                    start_nth(pending[e % 2])
                    pending[e % 2] += 2
    x_copy.wait()
    gw_copy.wait()

    x = x_v[...].astype(F32)
    x = jnp.concatenate([x, x], axis=0)
    x16 = x.astype(BF16)
    row = lax.broadcasted_iota(jnp.int32, (2 * B, DH), 0)
    row_pr = lax.broadcasted_iota(jnp.int32, (2 * B, PR), 0)

    def project_q(j):
        for g in range(2):
            q = []
            for hh in (2 * g, 2 * g + 1):
                cols = pl.ds(_aligned((hh * NJ + j) * DH, DH), DH)
                q.append(jnp.dot(x16, wq_v[:, :, cols].reshape(D, DH), preferred_element_type=F32))
            q_v[j, g] = jnp.where(row < B, q[0], q[1])

    chunks = pl.cdiv(F // 2, DH)

    def ffn_chunk(i):
        half, c = i // chunks, i % chunks
        lo = lax.min(c * DH, F // 2 - DH)
        rows = pl.ds(pl.multiple_of(lo, 16), DH)
        g = lax.dot_general(x16, wg_v[half, rows, :], NT, preferred_element_type=F32)
        u = lax.dot_general(x16, wu_v[half, rows, :], NT, preferred_element_type=F32)
        col = lax.broadcasted_iota(jnp.int32, (2 * B, DH), 1)
        hidden = jnp.where(col >= c * DH - lo, g * jax.nn.sigmoid(g) * u, 0.0)
        ffn_v[...] += jnp.dot(hidden.astype(BF16), wd_v[half, rows, :], preferred_element_type=F32)

    ffn_v[...] = jnp.zeros(ffn_v.shape, F32)
    project_q(0)
    gw = gw_v[...].astype(F32)
    logit = sum(x[:B, c * DH:(c + 1) * DH] * gw[c:c + 1] for c in range(D // DH))
    gate = jax.nn.sigmoid(jnp.sum(logit, axis=-1, keepdims=True))

    def period(kv, j, i, product, rows):
        tiles = [None, None]
        for s0 in range(0, NS, JOB):
            streams = range(s0, s0 + JOB)
            for n in streams:
                dma("wait", kv, j, i, 2 * n + 1)
                dma("start", kv, j, i, 2 * (n + AHEAD) + 1)
                if n > s0:
                    dma("start", kv, j, i, 2 * (n + 1 + AHEAD))
            for n in streams:
                dma("wait", kv, j, i, 2 * n)
            for n in streams:
                g, r = divmod(n, 2 * B)
                res = product(g, caches[kv][1][n, pl.ds(_aligned(i * PR, PR), PR), :])
                tiles[g] = res if tiles[g] is None else jnp.where(rows == r, res, tiles[g])
            dma("start", kv, j, i, 2 * (s0 + JOB + 1 + AHEAD))
        return tiles

    def fold(op, acc, tile):
        for c in range(PR // DH):
            acc = op(acc, tile[:, c * DH:(c + 1) * DH])
        return acc

    def run_periods(step, carry):
        looped = NP - 3
        carry = lax.fori_loop(0, looped, step, carry)
        for i in range(looped, NP):
            carry = step(i, carry)
        return carry

    def head_step(j, carry):
        q = [q_v[j, g].astype(BF16) for g in range(2)]

        def key_period(i, m):
            scores = period(
                0, j, i, lambda g, k: lax.dot_general(q[g], k, NT, preferred_element_type=F32), row_pr)
            if not isinstance(i, int):
                pl.when(jnp.logical_and(j == 0, i < 2 * chunks))(lambda: ffn_chunk(i))
                pl.when(jnp.logical_and(j < NJ - 1, i == 2 * chunks))(
                    lambda: project_q(lax.min(j + 1, NJ - 1)))
            scores = [s * DH ** -0.5 for s in scores]
            for g in range(2):
                s_v[i, g] = scores[g]
            return tuple(fold(jnp.maximum, m[g], scores[g]) for g in range(2))

        m = run_periods(key_period, (jnp.full((2 * B, DH), -jnp.inf, F32),) * 2)
        m = [jnp.max(t, axis=-1, keepdims=True) for t in m]
        k_v[:, pl.ds(0, SHIFT), :] = k_v[:, pl.ds(SK, SHIFT), :]

        def value_period(i, carry):
            total, acc = carry
            p = [jnp.exp(s_v[i, g] - m[g]) for g in range(2)]
            total = tuple(fold(jnp.add, total[g], p[g]) for g in range(2))
            p = [t.astype(BF16) for t in p]
            out = period(1, j, i, lambda g, v: jnp.dot(p[g], v, preferred_element_type=F32), row)
            return total, tuple(acc[g] + out[g] for g in range(2))

        zeros = (jnp.zeros((2 * B, DH), F32),) * 2
        total, acc = run_periods(value_period, (zeros, zeros))
        heads = []
        for g in range(2):
            o = acc[g] / jnp.sum(total[g], axis=-1, keepdims=True)
            heads += [jnp.where(row < B, o, 0.0), jnp.where(row < B, 0.0, o)]

        def project_out(y):
            v_v[:, pl.ds(0, SHIFT), :] = v_v[:, pl.ds(SK, SHIFT), :]
            jj = lax.min(j, NJ - 2)
            rows = pl.ds(pl.multiple_of((jj % 4) * DH, DH), DH)
            w = wo_v[:, jj // 4, rows, :].reshape(NH * DH, D)
            o = jnp.concatenate(heads, axis=-1).astype(BF16)
            return y + jnp.dot(o, w, preferred_element_type=F32)

        return lax.cond(j < NJ - 1, project_out, lambda y: y, carry[0]), tuple(heads)

    for n in range(2):
        dma("start", 0, 0, 0, 2 * (n + AHEAD))
    y, heads = lax.fori_loop(
        0, NJ, head_step, (jnp.zeros((2 * B, D), F32), (jnp.zeros((2 * B, DH), F32),) * NH))

    y = gate * (y[:B] + y[B:]) + (1.0 - gate) * ffn_v[:B]
    heads = [gate * (o[:B] + o[B:]) for o in heads]
    for t, n in enumerate(WO_TAIL):
        lo = sum(WO_TAIL[:t])
        o = jnp.concatenate(heads[lo:lo + n], axis=-1).astype(BF16)
        ffn_v[:B] = y
        wo_tail_copy(t).wait()
        w = wo_v[lo:lo + n, 1, pl.ds(3 * DH, DH), :].reshape(n * DH, D)
        y = y + jnp.dot(o, w, preferred_element_type=F32)
    out_v[...] = y.astype(out_v.dtype)
    out_copy = pltpu.make_async_copy(out_v, out_hbm, io_sem.at[2])
    out_copy.start()
    out_copy.wait()


@jax.jit
def pallas_gated_mix__mha_block_cached__swiglu_ffn__decode_kernel(
    A_x: jax.Array,
    A_k_cache: jax.Array,
    A_v_cache: jax.Array,
    A_wq: jax.Array,
    A_wo: jax.Array,
    B_x: jax.Array,
    B_w_gate: jax.Array,
    B_w_up: jax.Array,
    B_w_down: jax.Array,
    gate_w: jax.Array,
):
    hbm = pl.BlockSpec(memory_space=pltpu.HBM)
    cache_shape = (B, NH, NJ * SK, DH)
    wq_shape = (8, D // 8, H * DH)
    wo_shape = (NH, 2, NJ * DH // 2, D)
    ffn_shape = (2, F // 2, D)
    out = pl.pallas_call(
        _kernel,
        in_specs=[hbm] * 9,
        out_specs=hbm,
        out_shape=jax.ShapeDtypeStruct((B, D), BF16),
        scratch_shapes=[
            pltpu.VMEM((B, D), BF16),
            pltpu.VMEM((D // DH, DH), BF16),
            pltpu.VMEM(wq_shape, BF16),
            pltpu.VMEM(wo_shape, BF16),
            pltpu.VMEM(ffn_shape, BF16),
            pltpu.VMEM(ffn_shape, BF16),
            pltpu.VMEM(ffn_shape, BF16),
            pltpu.VMEM((NS, SK + SHIFT, DH), BF16),
            pltpu.VMEM((NS, SK + SHIFT, DH), BF16),
            pltpu.VMEM((NJ, 2, 2 * B, DH), F32),
            pltpu.VMEM((NP, 2, 2 * B, PR), F32),
            pltpu.VMEM((2 * B, D), F32),
            pltpu.VMEM((B, D), BF16),
            pltpu.SemaphoreType.DMA((RING * 2 * NS,)),
            pltpu.SemaphoreType.DMA((W_RING,)),
            pltpu.SemaphoreType.DMA((3,)),
        ],
        compiler_params=pltpu.CompilerParams(
            vmem_limit_bytes=64 * 1024 * 1024,
            disable_semaphore_checks=True,
        ),
        name="gated_mix_decode",
    )(
        A_x.reshape(B, D),
        A_k_cache.reshape(cache_shape),
        A_v_cache.reshape(cache_shape),
        A_wq.reshape(wq_shape),
        A_wo.reshape(wo_shape),
        B_w_gate.T.reshape(ffn_shape),
        B_w_up.T.reshape(ffn_shape),
        B_w_down.reshape(ffn_shape),
        gate_w.reshape(D // DH, DH),
    )
    return out.reshape(B, 1, D)
```

```python
import functools

import jax
import jax.numpy as jnp
from jax import lax
import jax.experimental.pallas as pl
import jax.experimental.pallas.tpu as pltpu

B, D, H, SK, DH, F = 4, 512, 32, 4096, 128, 1376

NH = 4
NS = B * NH
NJ = H // NH
PR = 256
NP = SK // PR
SHORT = 32
SHIFT = 96
AHEAD = 24
JOB = 4
RING = 4
W_AHEAD = 16
W_RING = 64
START_GAP = 6
WO_TAIL = (3, 1)

NT = (((1,), (1,)), ((), ()))
F32, BF16 = jnp.float32, jnp.bfloat16


def _aligned(i, n):
    return i if isinstance(i, int) else pl.multiple_of(i, n)


def _kernel(x_hbm, k_hbm, v_hbm, wq_hbm, wo_hbm, wg_hbm, wu_hbm, wd_hbm, gw_hbm, out_hbm,
            x_v, gw_v, wq_v, wo_v, wg_v, wu_v, wd_v, k_v, v_v, q_v, s_v, ffn_v, out_v,
            kv_sem, w_sem, io_sem):
    caches = ((k_hbm, k_v), (v_hbm, v_v))

    def cache_copy(kv, j, i, e, clip=False):
        hbm, vmem = caches[kv]
        n = e // 2
        r = i * PR + SHIFT + (0, SHORT)[e % 2]
        rows = SK - r if clip else (SHORT, PR - SHORT)[e % 2]
        return pltpu.make_async_copy(
            hbm.at[n % B, n // B, pl.ds(_aligned(j * SK + r, 16), rows)],
            vmem.at[n, pl.ds(_aligned(r, 16), rows)],
            kv_sem.at[(i % RING) * 2 * NS + e])

    def cache_op(op, kv, j, i, e):
        def run(j, clip):
            copy = cache_copy(kv, j, i, e, clip)
            copy.wait() if op == "wait" else copy.start(priority=e % 2)

        if isinstance(i, int) and i == NP - 1 and e % 2:
            pl.when(j < NJ - 1)(lambda: run(lax.min(j, NJ - 2), False))
            pl.when(j == NJ - 1)(lambda: run(NJ - 1, True))
        else:
            run(j, False)

    def wo_tail_copy(t):
        idx = (pl.ds(sum(WO_TAIL[:t]), WO_TAIL[t]), 1, pl.ds(3 * DH, DH))
        return pltpu.make_async_copy(wo_hbm.at[idx], wo_v.at[idx], w_sem.at[t])

    def dma(op, kv, j, i, e):
        di, e = divmod(e, 2 * NS)
        if not isinstance(i, int) or i + di < NP:
            cache_op(op, kv, j, i + di, e)
        elif kv == 0:
            cache_op(op, 1, j, i + di - NP, e)
        else:
            pl.when(j < NJ - 1)(
                functools.partial(cache_op, op, 0, lax.min(j + 1, NJ - 1), i + di - NP, e))
            t = (i + di - NP) * NS + e // 2
            if op == "start" and e % 2 and t < len(WO_TAIL):
                pl.when(j == NJ - 1)(lambda: wo_tail_copy(t).start(priority=1))

    def weight_slices(section, u):
        out = []

        def ffn(t):
            rows = pl.ds(_aligned(t * 16, 16), 16)
            out.append((wu_hbm, wu_v, (pl.ds(0, 1), rows)))
            out.append((wg_hbm, wg_v, (pl.ds(0, 2), rows)))
            out.append((wu_hbm, wu_v, (pl.ds(1, 1), rows)))
            out.append((wd_hbm, wd_v, (pl.ds(0, 2), rows)))

        if section < 2:
            t = u + (0, 24)[section]
            q_rows = pl.ds(_aligned((t // 4) * 8, 8), 8)
            q_cols = pl.ds(_aligned((t % 4) * 1024, 1024), 1024)
            o_rows = pl.ds(_aligned(t * 16, 16), 16)
            for s in (0, 4):
                out.append((wq_hbm, wq_v, (pl.ds(s, 1), q_rows, q_cols)))
                out.append((wq_hbm, wq_v, (pl.ds(s + 1, 3), q_rows, q_cols)))
            for half in range(2 - section):
                out.append((wo_hbm, wo_v, (pl.ds(0, 1), half, o_rows)))
                out.append((wo_hbm, wo_v, (pl.ds(1, 3), half, o_rows)))
            for t in ((u,), (24 + 2 * u, 25 + 2 * u))[section]:
                ffn(t)
        else:
            for t in range(40, F // 32):
                ffn(t)
        out = [(src.at[idx], dst.at[idx]) for src, dst, idx in out]
        if section == 2:
            for hbm, vmem in caches:
                for hh in range(NH):
                    for b, nb in ((0, 1), (1, B - 1)):
                        out.append((hbm.at[pl.ds(b, nb), hh, pl.ds(0, SHIFT)],
                                    vmem.at[pl.ds(hh * B + b, nb), pl.ds(0, SHIFT)]))
        return out

    steps = (24, 8, 1)
    width = [len(weight_slices(s, 0)) for s in range(3)]
    first = [sum(w * n for w, n in zip(width[:s], steps[:s])) for s in range(4)]
    n_weight = first[-1]

    def weight_copy(section, u, e):
        src, dst = weight_slices(section, u)[e]
        return pltpu.make_async_copy(
            src, dst, w_sem.at[(first[section] + u * width[section] + e) % W_RING])

    def start_nth(t):
        if t < n_weight:
            s = max(k for k in range(3) if first[k] <= t)
            weight_copy(s, *divmod(t - first[s], width[s])).start(priority=t % 2)
        else:
            cache_op("start", 0, 0, *divmod(t - n_weight, 2 * NS))

    x_copy = pltpu.make_async_copy(x_hbm, x_v, io_sem.at[0])
    gw_copy = pltpu.make_async_copy(gw_hbm, gw_v, io_sem.at[1])
    for t in range(1, 2 * W_AHEAD, 2):
        start_nth(t)
    for t in range(0, 2 * W_AHEAD, 2):
        @pl.loop(0, START_GAP)
        def _(_):
            ffn_v[...] = jnp.zeros(ffn_v.shape, F32)
        start_nth(t)
    x_copy.start()
    gw_copy.start()
    pending = [2 * W_AHEAD, 2 * W_AHEAD + 1]
    for s in range(3):
        looped = max(0, steps[s] - pl.cdiv(2 * W_AHEAD, width[s]))
        if looped:
            @pl.loop(0, looped)
            def _(u):
                for e in range(width[s]):
                    weight_copy(s, u, e).wait()
                    du, e2 = divmod(e + 2 * W_AHEAD, width[s])
                    weight_copy(s, u + du, e2).start(priority=e % 2)
            pending = [t + looped * width[s] for t in pending]
        for u in range(looped, steps[s]):
            for e in range(width[s]):
                weight_copy(s, u, e).wait()
                t = first[s] + u * width[s] + e
                upto = t + 2 * W_AHEAD if t + 2 < n_weight else n_weight + 2 * AHEAD - 1
                while pending[e % 2] <= upto:
                    start_nth(pending[e % 2])
                    pending[e % 2] += 2
    x_copy.wait()
    gw_copy.wait()

    x = x_v[...].astype(F32)
    x = jnp.concatenate([x, x], axis=0)
    x16 = x.astype(BF16)
    row = lax.broadcasted_iota(jnp.int32, (2 * B, DH), 0)
    row_pr = lax.broadcasted_iota(jnp.int32, (2 * B, PR), 0)

    def project_q(j):
        for g in range(2):
            q = []
            for hh in (2 * g, 2 * g + 1):
                cols = pl.ds(_aligned((hh * NJ + j) * DH, DH), DH)
                q.append(jnp.dot(x16, wq_v[:, :, cols].reshape(D, DH), preferred_element_type=F32))
            q_v[j, g] = jnp.where(row < B, q[0], q[1])

    chunks = pl.cdiv(F // 2, DH)

    def ffn_chunk(i):
        half, c = lax.min(i // chunks, 1), i % chunks
        lo = lax.min(c * DH, F // 2 - DH)
        rows = pl.ds(pl.multiple_of(lo, 16), DH)
        g = lax.dot_general(x16, wg_v[half, rows, :], NT, preferred_element_type=F32)
        u = lax.dot_general(x16, wu_v[half, rows, :], NT, preferred_element_type=F32)
        col = lax.broadcasted_iota(jnp.int32, (2 * B, DH), 1)
        hidden = jnp.where(col >= c * DH - lo, g * jax.nn.sigmoid(g) * u, 0.0)
        ffn_v[...] += jnp.dot(hidden.astype(BF16), wd_v[half, rows, :], preferred_element_type=F32)

    project_q(0)
    gw = gw_v[...].astype(F32)
    logit = sum(x[:B, c * DH:(c + 1) * DH] * gw[c:c + 1] for c in range(D // DH))
    gate = jax.nn.sigmoid(jnp.sum(logit, axis=-1, keepdims=True))

    def period(kv, j, i, product, rows):
        tiles = [None, None]
        for s0 in range(0, NS, JOB):
            streams = range(s0, s0 + JOB)
            for n in streams:
                dma("wait", kv, j, i, 2 * n + 1)
                dma("start", kv, j, i, 2 * (n + AHEAD) + 1)
                if n > s0:
                    dma("start", kv, j, i, 2 * (n + 1 + AHEAD))
            for n in streams:
                dma("wait", kv, j, i, 2 * n)
            for n in streams:
                g, r = divmod(n, 2 * B)
                res = product(g, caches[kv][1][n, pl.ds(_aligned(i * PR, PR), PR), :])
                tiles[g] = res if tiles[g] is None else jnp.where(rows == r, res, tiles[g])
            dma("start", kv, j, i, 2 * (s0 + JOB + 1 + AHEAD))
        return tiles

    def fold(op, acc, tile):
        for c in range(PR // DH):
            acc = op(acc, tile[:, c * DH:(c + 1) * DH])
        return acc

    def run_periods(step, carry):
        looped = NP - 3
        carry = lax.fori_loop(0, looped, step, carry)
        for i in range(looped, NP):
            carry = step(i, carry)
        return carry

    def head_step(j, carry):
        q = [q_v[j, g].astype(BF16) for g in range(2)]

        def key_period(i, m):
            scores = period(
                0, j, i, lambda g, k: lax.dot_general(q[g], k, NT, preferred_element_type=F32), row_pr)
            if not isinstance(i, int):
                pl.when(jnp.logical_and(j == 0, i < 2 * chunks))(lambda: ffn_chunk(i))
                pl.when(jnp.logical_and(j < NJ - 1, i == 2 * chunks))(
                    lambda: project_q(lax.min(j + 1, NJ - 1)))
            scores = [s * DH ** -0.5 for s in scores]
            for g in range(2):
                s_v[i, g] = scores[g]
            return tuple(fold(jnp.maximum, m[g], scores[g]) for g in range(2))

        m = run_periods(key_period, (jnp.full((2 * B, DH), -jnp.inf, F32),) * 2)
        m = [jnp.max(t, axis=-1, keepdims=True) for t in m]
        k_v[:, pl.ds(0, SHIFT), :] = k_v[:, pl.ds(SK, SHIFT), :]

        def value_period(i, carry):
            total, acc = carry
            p = [jnp.exp(s_v[i, g] - m[g]) for g in range(2)]
            total = tuple(fold(jnp.add, total[g], p[g]) for g in range(2))
            p = [t.astype(BF16) for t in p]
            out = period(1, j, i, lambda g, v: jnp.dot(p[g], v, preferred_element_type=F32), row)
            return total, tuple(acc[g] + out[g] for g in range(2))

        zeros = (jnp.zeros((2 * B, DH), F32),) * 2
        total, acc = run_periods(value_period, (zeros, zeros))
        heads = []
        for g in range(2):
            o = acc[g] / jnp.sum(total[g], axis=-1, keepdims=True)
            heads += [jnp.where(row < B, o, 0.0), jnp.where(row < B, 0.0, o)]

        def project_out(y):
            v_v[:, pl.ds(0, SHIFT), :] = v_v[:, pl.ds(SK, SHIFT), :]
            jj = lax.min(j, NJ - 2)
            rows = pl.ds(pl.multiple_of((jj % 4) * DH, DH), DH)
            w = wo_v[:, jj // 4, rows, :].reshape(NH * DH, D)
            o = jnp.concatenate(heads, axis=-1).astype(BF16)
            return y + jnp.dot(o, w, preferred_element_type=F32)

        return lax.cond(j < NJ - 1, project_out, lambda y: y, carry[0]), tuple(heads)

    for n in range(2):
        dma("start", 0, 0, 0, 2 * (n + AHEAD))
    y, heads = lax.fori_loop(
        0, NJ, head_step, (jnp.zeros((2 * B, D), F32), (jnp.zeros((2 * B, DH), F32),) * NH))

    y = gate * (y[:B] + y[B:]) + (1.0 - gate) * ffn_v[:B]
    heads = [gate * (o[:B] + o[B:]) for o in heads]
    for t, n in enumerate(WO_TAIL):
        lo = sum(WO_TAIL[:t])
        o = jnp.concatenate(heads[lo:lo + n], axis=-1).astype(BF16)
        ffn_v[:B] = y
        wo_tail_copy(t).wait()
        w = wo_v[lo:lo + n, 1, pl.ds(3 * DH, DH), :].reshape(n * DH, D)
        y = y + jnp.dot(o, w, preferred_element_type=F32)
    out_v[...] = y.astype(out_v.dtype)
    out_copy = pltpu.make_async_copy(out_v, out_hbm, io_sem.at[2])
    out_copy.start()
    out_copy.wait()


@jax.jit
def pallas_gated_mix__mha_block_cached__swiglu_ffn__decode_kernel(
    A_x: jax.Array,
    A_k_cache: jax.Array,
    A_v_cache: jax.Array,
    A_wq: jax.Array,
    A_wo: jax.Array,
    B_x: jax.Array,
    B_w_gate: jax.Array,
    B_w_up: jax.Array,
    B_w_down: jax.Array,
    gate_w: jax.Array,
):
    hbm = pl.BlockSpec(memory_space=pltpu.HBM)
    cache_shape = (B, NH, NJ * SK, DH)
    wq_shape = (8, D // 8, H * DH)
    wo_shape = (NH, 2, NJ * DH // 2, D)
    ffn_shape = (2, F // 2, D)
    out = pl.pallas_call(
        _kernel,
        in_specs=[hbm] * 9,
        out_specs=hbm,
        out_shape=jax.ShapeDtypeStruct((B, D), BF16),
        scratch_shapes=[
            pltpu.VMEM((B, D), BF16),
            pltpu.VMEM((D // DH, DH), BF16),
            pltpu.VMEM(wq_shape, BF16),
            pltpu.VMEM(wo_shape, BF16),
            pltpu.VMEM(ffn_shape, BF16),
            pltpu.VMEM(ffn_shape, BF16),
            pltpu.VMEM(ffn_shape, BF16),
            pltpu.VMEM((NS, SK + SHIFT, DH), BF16),
            pltpu.VMEM((NS, SK + SHIFT, DH), BF16),
            pltpu.VMEM((NJ, 2, 2 * B, DH), F32),
            pltpu.VMEM((NP, 2, 2 * B, PR), F32),
            pltpu.VMEM((2 * B, D), F32),
            pltpu.VMEM((B, D), BF16),
            pltpu.SemaphoreType.DMA((RING * 2 * NS,)),
            pltpu.SemaphoreType.DMA((W_RING,)),
            pltpu.SemaphoreType.DMA((3,)),
        ],
        compiler_params=pltpu.CompilerParams(
            vmem_limit_bytes=64 * 1024 * 1024,
            disable_semaphore_checks=True,
        ),
        name="gated_mix_decode",
    )(
        A_x.reshape(B, D),
        A_k_cache.reshape(cache_shape),
        A_v_cache.reshape(cache_shape),
        A_wq.reshape(wq_shape),
        A_wo.reshape(wo_shape),
        B_w_gate.T.reshape(ffn_shape),
        B_w_up.T.reshape(ffn_shape),
        B_w_down.reshape(ffn_shape),
        gate_w.reshape(D // DH, DH),
    )
    return out.reshape(B, 1, D)
```
